```python
import os as _os
_os.environ.setdefault('JAX_PLATFORMS', 'cpu')
import jax
import jax.numpy as jnp

def _softmax(x, axis=-1):
    return jax.nn.softmax(x, axis=axis)

def _gelu(x):
    return jax.nn.gelu(x, approximate=True)

def _silu(x):
    return jax.nn.silu(x)

def _sigmoid(x):
    return jax.nn.sigmoid(x)

def _layernorm(x, axis=-1, eps=1e-05):
    m = jnp.mean(x, axis=axis, keepdims=True)
    v = jnp.var(x, axis=axis, keepdims=True)
    return (x - m) / jnp.sqrt(v + eps)

def _scatter_add(tgt, idx, src, axis=0):
    return tgt.at[idx].add(src)

def _segment_sum(src, seg, n):
    return jax.ops.segment_sum(src, seg, n)

class _Rng:

    def __init__(self, key):
        self._k = key

    def _next(self):
        self._k, sub = jax.random.split(self._k)
        return sub

    def normal(self, shape):
        return jax.random.normal(self._next(), shape, dtype=jnp.bfloat16)

    def randint(self, lo, hi, shape):
        return jax.random.randint(self._next(), shape, lo, hi, dtype=jnp.int32)

    def uniform(self, shape, lo=0.0, hi=1.0):
        return jax.random.uniform(self._next(), shape, jnp.bfloat16, lo, hi)

    def permutation(self, n):
        return jax.random.permutation(self._next(), n)
kernel_name = 'adaLN_cond__mha_block_cached__geglu_ffn__prompt'

def setup_inputs():
    _rng = _Rng(jax.random.key(int.from_bytes(__import__("os").urandom(4), "little")))
    _w = lambda a: (lambda t: t.astype(jnp.bfloat16) if jnp.issubdtype(t.dtype, jnp.floating) else t)(jnp.asarray(a))

    def _A_setup():
        B, Sq, D = (1, 2048, 512)
        H, Sk, Dh = (32, 2048, 128)
        return {'x': _w((lambda *s: _rng.normal(s) * 0.05)(B, Sq, D)), 'k_cache': _w((lambda *s: _rng.normal(s) * 3.2)(B, H, Sk, Dh)), 'v_cache': _w((lambda *s: _rng.normal(s) * 0.4)(B, H, Sk, Dh)), 'wq': _w((lambda *s: _rng.normal(s) * 1.6)(D, H * Dh) * D ** (-0.5)), 'wo': _w((lambda *s: _rng.normal(s) * 0.4)(H * Dh, D) * (H * Dh) ** (-0.5))}
    _A_in = _A_setup()

    def _B_setup():
        B, S, D, F = (1, 2048, 512, 1792)
        return {'x': _w((lambda *s: _rng.normal(s) * 0.05)(B, S, D)), 'w_gate': _w((lambda *s: _rng.normal(s) * 0.05)(D, F)), 'w_up': _w((lambda *s: _rng.normal(s) * 0.05)(D, F)), 'w_down': _w((lambda *s: _rng.normal(s) * 0.05)(F, D))}
    _B_in = _B_setup()
    return {'A_x': _A_in['x'], 'A_k_cache': _A_in['k_cache'], 'A_v_cache': _A_in['v_cache'], 'A_wq': _A_in['wq'], 'A_wo': _A_in['wo'], 'B_x': _B_in['x'], 'B_w_gate': _B_in['w_gate'], 'B_w_up': _B_in['w_up'], 'B_w_down': _B_in['w_down'], 'c': _w((lambda *s: _rng.normal(s) * 0.05)(1, 512) * 8.0), 'w_mod': _w((lambda *s: _rng.normal(s) * 0.05)(512, 6 * 512) * 512 ** (-0.5) * 8.0)}

def reference(A_x, A_k_cache, A_v_cache, A_wq, A_wo, B_x, B_w_gate, B_w_up, B_w_down, c, w_mod):

    def _A_ref(x, k_cache, v_cache, wq, wo):
        B, Sq, D = x.shape
        H, Dh = (32, 128)
        q = (lambda x, *d: x.transpose(*d))((x @ wq).reshape(B, Sq, H, Dh), 0, 2, 1, 3)
        scores = jnp.einsum('bhqd,bhkd->bhqk', q, k_cache) * Dh ** (-0.5)
        p = _softmax(scores, axis=-1)
        o = jnp.einsum('bhqk,bhkd->bhqd', p, v_cache)
        return (lambda x, *d: x.transpose(*d))(o, 0, 2, 1, 3).reshape(B, Sq, H * Dh) @ wo

    def _B_ref(x, w_gate, w_up, w_down):
        return _gelu(x @ w_gate) * (x @ w_up) @ w_down
    x = A_x
    mod = (_silu(c) @ w_mod).reshape(c.shape[0], 6, 1, -1)
    sa, ca, ga, sb, cb, gb = (mod[:, 0].copy(), mod[:, 1].copy(), mod[:, 2].copy(), mod[:, 3].copy(), mod[:, 4].copy(), mod[:, 5].copy())
    h = _layernorm(x, axis=-1) * (1 + ca) + sa
    x = x + ga * _A_ref(h, A_k_cache, A_v_cache, A_wq, A_wo)
    h = _layernorm(x, axis=-1) * (1 + cb) + sb
    x = x + gb * _B_ref(h, B_w_gate, B_w_up, B_w_down)
    return x
```

```python
import jax
import jax.numpy as jnp
import jax.experimental.pallas as pl
import jax.experimental.pallas.tpu as pltpu

F32 = jnp.float32
BF16 = jnp.bfloat16
LOG2E = 1.4426950408889634

NT = (((1,), (1,)), ((), ()))


def _ln(x):
    m = jnp.mean(x, axis=-1, keepdims=True)
    xc = x - m
    v = jnp.mean(xc * xc, axis=-1, keepdims=True)
    return xc * jax.lax.rsqrt(v + 1e-5)


def _gelu(x):
    return 0.5 * x * (1.0 + jnp.tanh(0.7978845608028654 * (x + 0.044715 * (x * x * x))))


def _tilered(s, op):
    n = s.shape[1] // 128
    m = s[:, 0:128]
    for t in range(1, n):
        m = op(m, s[:, t * 128:(t + 1) * 128])
    return m


@jax.jit
def pallas_adaLN_cond__mha_block_cached__geglu_ffn__prompt_kernel(
    A_x: jax.Array,
    A_k_cache: jax.Array,
    A_v_cache: jax.Array,
    A_wq: jax.Array,
    A_wo: jax.Array,
    B_x: jax.Array,
    B_w_gate: jax.Array,
    B_w_up: jax.Array,
    B_w_down: jax.Array,
    c: jax.Array,
    w_mod: jax.Array,
):
    B, S, D = A_x.shape
    _, H, SK, DH = A_k_cache.shape
    FF = B_w_gate.shape[1]
    R, CH, BF, FU, XCH = 256, 512, 256, 2, 8
    NB, NC, NF, XR = S // R, SK // CH, S // BF, S // XCH
    QS = DH ** -0.5 * LOG2E

    def kernel(x_hbm, c_hbm, wmod_hbm, wq_hbm, k_hbm, v_hbm, wo_hbm, wg_hbm, wu_hbm, wd_hbm, o_hbm,
               x_v, c_v, wmod_v, wq_v, k_v, v_v, wo_v, wg_v, wu_v, wd_v, h_scr, acc_scr, q_scr, mod_scr, o_v,
               sem_x, sem_m, sem_h, sem_f, sem_o):

        def cp_k(h, slot): return pltpu.make_async_copy(k_hbm.at[h], k_v.at[slot], sem_h.at[0, slot])
        def cp_v(h, slot): return pltpu.make_async_copy(v_hbm.at[h], v_v.at[slot], sem_h.at[1, slot])
        def cp_wq(h, slot):
            return pltpu.make_async_copy(wq_hbm.at[:, pl.ds(pl.multiple_of(h * DH, DH), DH)], wq_v.at[slot], sem_h.at[2, slot])
        def cp_wo(h, slot):
            return pltpu.make_async_copy(wo_hbm.at[pl.ds(pl.multiple_of(h * DH, DH), DH), :], wo_v.at[slot], sem_h.at[3, slot])
        def cp_x(r): return pltpu.make_async_copy(x_hbm.at[pl.ds(r * XR, XR)], x_v.at[pl.ds(r * XR, XR)], sem_x.at[r])
        cp_c = pltpu.make_async_copy(c_hbm, c_v, sem_m.at[0])
        cp_m0 = pltpu.make_async_copy(wmod_hbm.at[:, 0:2 * D], wmod_v.at[:, 0:2 * D], sem_m.at[1])
        cp_m1 = pltpu.make_async_copy(wmod_hbm.at[:, 2 * D:6 * D], wmod_v.at[:, 2 * D:6 * D], sem_m.at[2])
        cp_f = [pltpu.make_async_copy(a, b, sem_f.at[j])
                for j, (a, b) in enumerate([(wg_hbm, wg_v), (wu_hbm, wu_v), (wd_hbm, wd_v)])]

        cp_c.start(); cp_m0.start()
        for r in range(XCH):
            cp_x(r).start()
        cp_wq(0, 0).start(); cp_k(0, 0).start(); cp_wq(1, 1).start(); cp_v(0, 0).start(); cp_wo(0, 0).start()
        cp_m1.start()
        cp_c.wait(); cp_m0.wait()
        cc = c_v[...].astype(F32)
        sc = jnp.broadcast_to((cc * jax.nn.sigmoid(cc)).astype(BF16), (16, D))
        mod_a = jnp.dot(sc, wmod_v[:, 0:2 * D], preferred_element_type=F32)
        sa = mod_a[0:1, 0:D]
        ca = mod_a[0:1, D:2 * D]
        for r in range(S // 256):
            if (r * 256) % XR == 0:
                cp_x(r * 256 // XR).wait()
            rows = pl.ds(r * 256, 256)
            hh_ = _ln(x_v[rows, :].astype(F32)) * (1.0 + ca) + sa
            h_scr[rows, :] = hh_.astype(BF16)
            acc_scr[rows, :] = jnp.zeros((256, D), F32)
        cp_m1.wait()
        mod_b = jnp.dot(sc, wmod_v[:, 2 * D:6 * D], preferred_element_type=F32)
        mod_scr[...] = mod_b[0:8]
        for cp in cp_f:
            cp.start()

        def qproj(i, slot):
            q = jnp.dot(h_scr[i * R:(i + 1) * R, :], wq_v[slot], preferred_element_type=F32)
            q_scr[i * R:(i + 1) * R, :] = (q * QS).astype(BF16)

        cp_wq(0, 0).wait()
        qproj(0, 0)

        def head(h, slot):
            nslot = 1 - slot
            hn = jnp.minimum(h + 1, H - 1)
            qs = h % 3
            qs1 = (h + 1) % 3
            qs2 = (h + 2) % 3
            cp_k(h, slot).wait(); cp_v(h, slot).wait(); cp_wo(h, slot).wait(); cp_wq(hn, qs1).wait()

            @pl.when(h + 1 < H)
            def _():
                cp_k(h + 1, nslot).start(); cp_v(h + 1, nslot).start(); cp_wo(h + 1, nslot).start()
                cp_wq(jnp.minimum(h + 2, H - 1), qs2).start()

            kk = k_v.at[slot]
            vv = v_v.at[slot]

            def wo_step(i, o):
                acc_scr[i * R:(i + 1) * R, :] += jnp.dot(o, wo_v[slot], preferred_element_type=F32)

            oprev = None
            for i in range(NB):
                qn = q_scr[i * R:(i + 1) * R, :]
                mx = None
                sl = []
                for j in range(NC):
                    sn = jax.lax.dot_general(qn, kk[j * CH:(j + 1) * CH, :], NT, preferred_element_type=F32)
                    t = _tilered(sn, jnp.maximum)
                    mx = t if mx is None else jnp.maximum(mx, t)
                    sl.append(sn)
                m = jnp.max(mx, axis=-1, keepdims=True)
                if oprev is not None:
                    wo_step(i - 1, oprev)
                if i + 1 < NB:
                    qproj(i + 1, qs)
                o = None
                lsum = None
                for j in range(NC):
                    p = jnp.exp2(sl[j] - m)
                    t = _tilered(p, jnp.add)
                    lsum = t if lsum is None else lsum + t
                    oc = jnp.dot(p.astype(BF16), vv[j * CH:(j + 1) * CH, :], preferred_element_type=F32)
                    o = oc if o is None else o + oc
                lsum = jnp.where(o != o, o, lsum)
                l = jnp.sum(lsum, axis=-1, keepdims=True)
                oprev = (o * (1.0 / l)).astype(BF16)
            qproj(0, qs1)
            wo_step(NB - 1, oprev)

        def body(hh, carry):
            head(2 * hh, 0)
            head(2 * hh + 1, 1)
            return carry
        jax.lax.fori_loop(0, H // 2, body, 0)

        for cp in cp_f:
            cp.wait()
        ga = mod_scr[0:1, 0:D]
        sb = mod_scr[0:1, D:2 * D]
        cb = mod_scr[0:1, 2 * D:3 * D]
        gb = mod_scr[0:1, 3 * D:4 * D]

        def cp_o(r):
            rows = pl.ds(pl.multiple_of(r * BF, BF), BF)
            return pltpu.make_async_copy(o_v.at[rows], o_hbm.at[rows], sem_o.at[r])

        def fbody(r, carry):
            rows = pl.ds(pl.multiple_of(r * BF, BF), BF)
            x1 = x_v[rows, :].astype(F32) + ga * acc_scr[rows, :]
            h2 = (_ln(x1) * (1.0 + cb) + sb).astype(BF16)
            g = jnp.dot(h2, wg_v[...], preferred_element_type=F32)
            u = jnp.dot(h2, wu_v[...], preferred_element_type=F32)
            a = (_gelu(g) * u).astype(BF16)
            y = jnp.dot(a, wd_v[...], preferred_element_type=F32)
            o_v[rows, :] = (x1 + gb * y).astype(BF16)
            cp_o(r).start()
            return carry
        jax.lax.fori_loop(0, NF, fbody, 0, unroll=FU)

        def wbody(r, carry):
            cp_o(r).wait()
            return carry
        jax.lax.fori_loop(0, NF, wbody, 0)

    x2 = A_x.reshape(S, D)
    k3 = A_k_cache.reshape(H, SK, DH)
    v3 = A_v_cache.reshape(H, SK, DH)
    hbm = pl.BlockSpec(memory_space=pl.ANY)
    out = pl.pallas_call(
        kernel,
        in_specs=[hbm] * 10,
        out_specs=hbm,
        out_shape=jax.ShapeDtypeStruct((S, D), BF16),
        scratch_shapes=[
            pltpu.VMEM((S, D), BF16), pltpu.VMEM((1, D), BF16), pltpu.VMEM((D, 6 * D), BF16),
            pltpu.VMEM((3, D, DH), BF16), pltpu.VMEM((2, SK, DH), BF16), pltpu.VMEM((2, SK, DH), BF16),
            pltpu.VMEM((2, DH, D), BF16),
            pltpu.VMEM((D, FF), BF16), pltpu.VMEM((D, FF), BF16), pltpu.VMEM((FF, D), BF16),
            pltpu.VMEM((S, D), BF16), pltpu.VMEM((S, D), F32), pltpu.VMEM((S, DH), BF16),
            pltpu.VMEM((8, 4 * D), F32), pltpu.VMEM((S, D), BF16),
            pltpu.SemaphoreType.DMA((XCH,)), pltpu.SemaphoreType.DMA((3,)), pltpu.SemaphoreType.DMA((4, 3)),
            pltpu.SemaphoreType.DMA((3,)), pltpu.SemaphoreType.DMA((NF,)),
        ],
        compiler_params=pltpu.CompilerParams(vmem_limit_bytes=100 * 1024 * 1024),
    )(x2, c, w_mod, A_wq, k3, v3, A_wo, B_w_gate, B_w_up, B_w_down)
    return out.reshape(B, S, D)
```

```python
import jax
import jax.numpy as jnp
import jax.experimental.pallas as pl
import jax.experimental.pallas.tpu as pltpu

F32 = jnp.float32
BF16 = jnp.bfloat16
LOG2E = 1.4426950408889634

NT = (((1,), (1,)), ((), ()))


def _ln(x):
    m = jnp.mean(x, axis=-1, keepdims=True)
    xc = x - m
    v = jnp.mean(xc * xc, axis=-1, keepdims=True)
    return xc * jax.lax.rsqrt(v + 1e-5)


def _gelu(x):
    return 0.5 * x * (1.0 + jnp.tanh(0.7978845608028654 * (x + 0.044715 * (x * x * x))))


def _tilered(s, op):
    n = s.shape[1] // 128
    m = s[:, 0:128]
    for t in range(1, n):
        m = op(m, s[:, t * 128:(t + 1) * 128])
    return m


@jax.jit
def pallas_adaLN_cond__mha_block_cached__geglu_ffn__prompt_kernel(
    A_x: jax.Array,
    A_k_cache: jax.Array,
    A_v_cache: jax.Array,
    A_wq: jax.Array,
    A_wo: jax.Array,
    B_x: jax.Array,
    B_w_gate: jax.Array,
    B_w_up: jax.Array,
    B_w_down: jax.Array,
    c: jax.Array,
    w_mod: jax.Array,
):
    B, S, D = A_x.shape
    _, H, SK, DH = A_k_cache.shape
    FF = B_w_gate.shape[1]
    R = 256
    CH = 512
    BF = 256
    XCH = 8
    NB, NC, NF, XR = S // R, SK // CH, S // BF, S // XCH
    QS = DH ** -0.5 * LOG2E

    def kernel(x_hbm, c_hbm, wmod_hbm, wq_hbm, k_hbm, v_hbm, wo_hbm, wg_hbm, wu_hbm, wd_hbm, o_hbm,
               x_v, c_v, wmod_v, wq_v, k_v, v_v, wo_v, wg_v, wu_v, wd_v,
               h_scr, acc_scr, q_scr, mod_scr, o_v, h2_scr, oc_scr, lc_scr,
               sem_x, sem_m, sem_h, sem_f, sem_o):

        def cp_k(h, slot):
            return pltpu.make_async_copy(k_hbm.at[h], k_v.at[slot], sem_h.at[0, slot])

        def cp_v(h, slot):
            return pltpu.make_async_copy(v_hbm.at[h], v_v.at[slot], sem_h.at[1, slot])

        def cp_wq(h, slot):
            cols = pl.ds(pl.multiple_of(h * DH, DH), DH)
            return pltpu.make_async_copy(wq_hbm.at[:, cols], wq_v.at[slot], sem_h.at[2, slot])

        def cp_wo(h, slot):
            rows = pl.ds(pl.multiple_of(h * DH, DH), DH)
            return pltpu.make_async_copy(wo_hbm.at[rows, :], wo_v.at[slot], sem_h.at[3, slot])

        def cp_x(r):
            rows = pl.ds(r * XR, XR)
            return pltpu.make_async_copy(x_hbm.at[rows], x_v.at[rows], sem_x.at[r])

        def cp_o(r):
            rows = pl.ds(pl.multiple_of(r * BF, BF), BF)
            return pltpu.make_async_copy(o_v.at[rows], o_hbm.at[rows], sem_o.at[r])

        cp_c = pltpu.make_async_copy(c_hbm, c_v, sem_m.at[0])
        cp_m0 = pltpu.make_async_copy(wmod_hbm.at[:, 0:2 * D], wmod_v.at[:, 0:2 * D], sem_m.at[1])
        cp_m1 = pltpu.make_async_copy(wmod_hbm.at[:, 2 * D:6 * D], wmod_v.at[:, 2 * D:6 * D], sem_m.at[2])
        cp_f = [pltpu.make_async_copy(src, dst, sem_f.at[j]) for j, (src, dst) in
                enumerate([(wg_hbm, wg_v), (wu_hbm, wu_v), (wd_hbm, wd_v)])]

        cp_c.start()
        cp_m0.start()
        for r in range(XCH):
            cp_x(r).start(1)
        for r in range(S // 256):
            acc_scr[pl.ds(r * 256, 256), :] = jnp.zeros((256, D), F32)
        wo_v[1] = jnp.zeros((DH, D), BF16)
        oc_scr[...] = jnp.zeros((R, DH), F32)
        lc_scr[...] = jnp.ones((R, DH), F32)
        cp_c.wait()
        cp_m0.wait()
        cf = c_v[...].astype(F32)
        sc = jnp.broadcast_to((cf * jax.nn.sigmoid(cf)).astype(BF16), (16, D))
        mod_a = jnp.dot(sc, wmod_v[:, 0:2 * D], preferred_element_type=F32)
        sa = mod_a[0:1, 0:D]
        ca1 = 1.0 + mod_a[0:1, D:2 * D]
        for r in range(XCH):
            cp_x(r).wait()
            if r == 5:
                cp_wq(0, 0).start(1)
                cp_k(0, 0).start(1)
                cp_v(0, 0).start(1)
                cp_wo(0, 0).start(1)
            rows = pl.ds(r * XR, XR)
            h_scr[rows, :] = (_ln(x_v[rows, :].astype(F32)) * ca1 + sa).astype(BF16)

        def qproj(i, slot):
            q = jnp.dot(h_scr[i * R:(i + 1) * R, :], wq_v[slot], preferred_element_type=F32)
            q_scr[i * R:(i + 1) * R, :] = (q * QS).astype(BF16)

        def wo_step(i, o, lsum, slot):
            lsum = jnp.where(o != o, o, lsum)
            l = jnp.sum(lsum, axis=-1, keepdims=True)
            on = (o * (1.0 / l)).astype(BF16)
            acc_scr[i * R:(i + 1) * R, :] += jnp.dot(on, wo_v[slot], preferred_element_type=F32)

        def head(h, slot, o, lsum):
            pslot = 1 - slot
            cp_k(h, slot).wait()
            cp_v(h, slot).wait()
            cp_wq(h, slot).wait()
            cp_wo(h, slot).wait()
            hn = jnp.minimum(h + 1, H - 1)
            cp_k(hn, pslot).start(1)
            cp_v(hn, pslot).start(1)
            cp_wq(hn, pslot).start(1)
            if slot == 1:
                @pl.when(h == 1)
                def _():
                    cp_m1.start(1)
                    for cp in cp_f:
                        cp.start(1)
            kk = k_v.at[slot]
            vv = v_v.at[slot]
            qproj(0, slot)
            wo_step(NB - 1, o, lsum, pslot)
            cp_wo(hn, pslot).start(1)
            for i in range(NB):
                qn = q_scr[i * R:(i + 1) * R, :]
                mx = None
                sl = []
                for j in range(NC):
                    sn = jax.lax.dot_general(qn, kk[j * CH:(j + 1) * CH, :], NT, preferred_element_type=F32)
                    t = _tilered(sn, jnp.maximum)
                    mx = t if mx is None else jnp.maximum(mx, t)
                    sl.append(sn)
                m = jnp.max(mx, axis=-1, keepdims=True)
                if i > 0:
                    wo_step(i - 1, o, lsum, slot)
                if i == 0:
                    qproj(1, slot)
                if i + 2 < NB:
                    qproj(i + 2, slot)
                o = None
                lsum = None
                for j in range(NC):
                    p = jnp.exp2(sl[j] - m)
                    t = _tilered(p, jnp.add)
                    lsum = t if lsum is None else lsum + t
                    oc = jnp.dot(p.astype(BF16), vv[j * CH:(j + 1) * CH, :], preferred_element_type=F32)
                    o = oc if o is None else o + oc
            return o, lsum

        def head_pair(g, carry):
            o, lsum = head(2 * g, 0, oc_scr[...], lc_scr[...])
            o, lsum = head(2 * g + 1, 1, o, lsum)
            oc_scr[...] = o
            lc_scr[...] = lsum
            return carry

        jax.lax.fori_loop(0, H // 2, head_pair, 0)

        cp_k(0, 0).wait()
        cp_v(0, 0).wait()
        cp_wq(0, 0).wait()
        cp_wo(0, 0).wait()
        cp_m1.wait()
        for cp in cp_f:
            cp.wait()
        wo_step(NB - 1, oc_scr[...], lc_scr[...], 1)

        mod_b = jnp.dot(sc, wmod_v[:, 2 * D:6 * D], preferred_element_type=F32)
        mod_scr[...] = mod_b[0:8]
        ga = mod_scr[0:1, 0:D]
        sb = mod_scr[0:1, D:2 * D]
        cb1 = 1.0 + mod_scr[0:1, 2 * D:3 * D]
        gb = mod_scr[0:1, 3 * D:4 * D]

        def x1_of(r):
            rows = pl.ds(pl.multiple_of(r * BF, BF), BF)
            return x_v[rows, :].astype(F32) + ga * acc_scr[rows, :]

        def pre(r):
            h2_scr[...] = (_ln(x1_of(r)) * cb1 + sb).astype(BF16)

        def ffn(r):
            rows = pl.ds(pl.multiple_of(r * BF, BF), BF)
            h2 = h2_scr[...]
            g = jnp.dot(h2, wg_v[...], preferred_element_type=F32)
            u = jnp.dot(h2, wu_v[...], preferred_element_type=F32)
            a = (_gelu(g) * u).astype(BF16)
            y = jnp.dot(a, wd_v[...], preferred_element_type=F32)
            o_v[rows, :] = (x1_of(r) + gb * y).astype(BF16)

        pre(0)

        def fbody(r, carry):
            ffn(r)
            pre(jnp.minimum(r + 1, NF - 1))
            cp_o(r).start()
            return carry

        jax.lax.fori_loop(0, NF, fbody, 0)

        def wbody(r, carry):
            cp_o(r).wait()
            return carry

        jax.lax.fori_loop(0, NF, wbody, 0)

    x2 = A_x.reshape(S, D)
    k3 = A_k_cache.reshape(H, SK, DH)
    v3 = A_v_cache.reshape(H, SK, DH)
    hbm = pl.BlockSpec(memory_space=pl.ANY)
    out = pl.pallas_call(
        kernel,
        in_specs=[hbm] * 10,
        out_specs=hbm,
        out_shape=jax.ShapeDtypeStruct((S, D), BF16),
        scratch_shapes=[
            pltpu.VMEM((S, D), BF16),
            pltpu.VMEM((1, D), BF16),
            pltpu.VMEM((D, 6 * D), BF16),
            pltpu.VMEM((2, D, DH), BF16),
            pltpu.VMEM((2, SK, DH), BF16),
            pltpu.VMEM((2, SK, DH), BF16),
            pltpu.VMEM((2, DH, D), BF16),
            pltpu.VMEM((D, FF), BF16),
            pltpu.VMEM((D, FF), BF16),
            pltpu.VMEM((FF, D), BF16),
            pltpu.VMEM((S, D), BF16),
            pltpu.VMEM((S, D), F32),
            pltpu.VMEM((S, DH), BF16),
            pltpu.VMEM((8, 4 * D), F32),
            pltpu.VMEM((S, D), BF16),
            pltpu.VMEM((BF, D), BF16),
            pltpu.VMEM((R, DH), F32),
            pltpu.VMEM((R, DH), F32),
            pltpu.SemaphoreType.DMA((XCH,)),
            pltpu.SemaphoreType.DMA((3,)),
            pltpu.SemaphoreType.DMA((4, 2)),
            pltpu.SemaphoreType.DMA((3,)),
            pltpu.SemaphoreType.DMA((NF,)),
        ],
        compiler_params=pltpu.CompilerParams(vmem_limit_bytes=100 * 1024 * 1024),
    )(x2, c, w_mod, A_wq, k3, v3, A_wo, B_w_gate, B_w_up, B_w_down)
    return out.reshape(B, S, D)
```

```python
import jax
import jax.numpy as jnp
import jax.experimental.pallas as pl
import jax.experimental.pallas.tpu as pltpu

F32 = jnp.float32
BF16 = jnp.bfloat16
LOG2E = 1.4426950408889634

NT = (((1,), (1,)), ((), ()))


def _ln(x):
    m = jnp.mean(x, axis=-1, keepdims=True)
    xc = x - m
    v = jnp.mean(xc * xc, axis=-1, keepdims=True)
    return xc * jax.lax.rsqrt(v + 1e-5)


def _gelu(x):
    return 0.5 * x * (1.0 + jnp.tanh(0.7978845608028654 * (x + 0.044715 * (x * x * x))))


def _tilered(s, op):
    n = s.shape[1] // 128
    m = s[:, 0:128]
    for t in range(1, n):
        m = op(m, s[:, t * 128:(t + 1) * 128])
    return m


@jax.jit
def pallas_adaLN_cond__mha_block_cached__geglu_ffn__prompt_kernel(
    A_x: jax.Array,
    A_k_cache: jax.Array,
    A_v_cache: jax.Array,
    A_wq: jax.Array,
    A_wo: jax.Array,
    B_x: jax.Array,
    B_w_gate: jax.Array,
    B_w_up: jax.Array,
    B_w_down: jax.Array,
    c: jax.Array,
    w_mod: jax.Array,
):
    B, S, D = A_x.shape
    _, H, SK, DH = A_k_cache.shape
    FF = B_w_gate.shape[1]
    R = 256
    CH = 512
    BF = 256
    XCH = 8
    NB, NC, NF, XR = S // R, SK // CH, S // BF, S // XCH
    QS = DH ** -0.5 * LOG2E

    def kernel(x_hbm, c_hbm, wmod_hbm, wq_hbm, k_hbm, v_hbm, wo_hbm, wg_hbm, wu_hbm, wd_hbm, o_hbm,
               x_v, c_v, wmod_v, wq_v, k_v, v_v, wo_v, wg_v, wu_v, wd_v,
               h_scr, acc_scr, q_scr, mod_scr, o_v, h2a_scr, h2b_scr, oc_scr, lc_scr,
               sem_x, sem_m, sem_h, sem_f, sem_o):

        def cp_k(h, slot):
            return pltpu.make_async_copy(k_hbm.at[h], k_v.at[slot], sem_h.at[0, slot])

        def cp_v(h, slot):
            return pltpu.make_async_copy(v_hbm.at[h], v_v.at[slot], sem_h.at[1, slot])

        def cp_wq(h, slot):
            cols = pl.ds(pl.multiple_of(h * DH, DH), DH)
            return pltpu.make_async_copy(wq_hbm.at[:, cols], wq_v.at[slot], sem_h.at[2, slot])

        def cp_wo(h, slot):
            rows = pl.ds(pl.multiple_of(h * DH, DH), DH)
            return pltpu.make_async_copy(wo_hbm.at[rows, :], wo_v.at[slot], sem_h.at[3, slot])

        def cp_x(r):
            rows = pl.ds(r * XR, XR)
            return pltpu.make_async_copy(x_hbm.at[rows], x_v.at[rows], sem_x.at[r])

        def cp_o(r):
            rows = pl.ds(pl.multiple_of(r * BF, BF), BF)
            return pltpu.make_async_copy(o_v.at[rows], o_hbm.at[rows], sem_o.at[r])

        cp_c = pltpu.make_async_copy(c_hbm, c_v, sem_m.at[0])
        cp_m0 = pltpu.make_async_copy(wmod_hbm.at[:, 0:2 * D], wmod_v.at[:, 0:2 * D], sem_m.at[1])
        cp_m1 = pltpu.make_async_copy(wmod_hbm.at[:, 2 * D:6 * D], wmod_v.at[:, 2 * D:6 * D], sem_m.at[2])
        cp_f = [pltpu.make_async_copy(src, dst, sem_f.at[j]) for j, (src, dst) in
                enumerate([(wg_hbm, wg_v), (wu_hbm, wu_v), (wd_hbm, wd_v)])]

        cp_c.start()
        cp_m0.start()
        for r in range(XCH):
            cp_x(r).start(1)
        for r in range(S // 256):
            acc_scr[pl.ds(r * 256, 256), :] = jnp.zeros((256, D), F32)
        wo_v[1] = jnp.zeros((DH, D), BF16)
        oc_scr[...] = jnp.zeros((R, DH), F32)
        lc_scr[...] = jnp.ones((R, DH), F32)
        cp_c.wait()
        cp_m0.wait()
        cf = c_v[...].astype(F32)
        sc = jnp.broadcast_to((cf * jax.nn.sigmoid(cf)).astype(BF16), (16, D))
        mod_a = jnp.dot(sc, wmod_v[:, 0:2 * D], preferred_element_type=F32)
        sa = mod_a[0:1, 0:D]
        ca1 = 1.0 + mod_a[0:1, D:2 * D]
        for r in range(XCH):
            cp_x(r).wait()
            if r == 5:
                cp_wq(0, 0).start(1)
                cp_k(0, 0).start(1)
                cp_v(0, 0).start(1)
                cp_wo(0, 0).start(1)
            rows = pl.ds(r * XR, XR)
            h_scr[rows, :] = (_ln(x_v[rows, :].astype(F32)) * ca1 + sa).astype(BF16)

        def qproj(i, slot):
            q = jnp.dot(h_scr[i * R:(i + 1) * R, :], wq_v[slot], preferred_element_type=F32)
            q_scr[i * R:(i + 1) * R, :] = (q * QS).astype(BF16)

        def wo_step(i, o, lsum, slot):
            lsum = jnp.where(o != o, o, lsum)
            l = jnp.sum(lsum, axis=-1, keepdims=True)
            on = (o * (1.0 / l)).astype(BF16)
            acc_scr[i * R:(i + 1) * R, :] += jnp.dot(on, wo_v[slot], preferred_element_type=F32)

        def head(h, slot, o, lsum):
            pslot = 1 - slot
            cp_k(h, slot).wait()
            cp_v(h, slot).wait()
            cp_wq(h, slot).wait()
            cp_wo(h, slot).wait()
            hn = jnp.minimum(h + 1, H - 1)
            if slot == 1:
                @pl.when(h == 1)
                def _():
                    cp_m1.start(1)
                    for cp in cp_f:
                        cp.start(1)
            kk = k_v.at[slot]
            vv = v_v.at[slot]
            qproj(0, slot)
            wo_step(NB - 1, o, lsum, pslot)
            cp_wo(hn, pslot).start(1)
            for i in range(NB):
                qn = q_scr[i * R:(i + 1) * R, :]
                mx = None
                sl = []
                for j in range(NC):
                    sn = jax.lax.dot_general(qn, kk[j * CH:(j + 1) * CH, :], NT, preferred_element_type=F32)
                    t = _tilered(sn, jnp.maximum)
                    mx = t if mx is None else jnp.maximum(mx, t)
                    sl.append(sn)
                m = jnp.max(mx, axis=-1, keepdims=True)
                if i > 0:
                    wo_step(i - 1, o, lsum, slot)
                if i == 0:
                    qproj(1, slot)
                if i + 2 < NB:
                    qproj(i + 2, slot)
                if i == 0:
                    cp_k(hn, pslot).start(1)
                    cp_v(hn, pslot).start(1)
                    cp_wq(hn, pslot).start(1)
                o = None
                lsum = None
                for j in range(NC):
                    p = jnp.exp2(sl[j] - m)
                    t = _tilered(p, jnp.add)
                    lsum = t if lsum is None else lsum + t
                    oc = jnp.dot(p.astype(BF16), vv[j * CH:(j + 1) * CH, :], preferred_element_type=F32)
                    o = oc if o is None else o + oc
            return o, lsum

        def head_pair(g, carry):
            o, lsum = head(2 * g, 0, oc_scr[...], lc_scr[...])
            o, lsum = head(2 * g + 1, 1, o, lsum)
            oc_scr[...] = o
            lc_scr[...] = lsum
            return carry

        jax.lax.fori_loop(0, H // 2, head_pair, 0)

        cp_k(0, 0).wait()
        cp_v(0, 0).wait()
        cp_wq(0, 0).wait()
        cp_wo(0, 0).wait()
        cp_m1.wait()
        for cp in cp_f:
            cp.wait()
        wo_step(NB - 1, oc_scr[...], lc_scr[...], 1)

        mod_b = jnp.dot(sc, wmod_v[:, 2 * D:6 * D], preferred_element_type=F32)
        mod_scr[...] = mod_b[0:8]
        ga = mod_scr[0:1, 0:D]
        sb = mod_scr[0:1, D:2 * D]
        cb1 = 1.0 + mod_scr[0:1, 2 * D:3 * D]
        gb = mod_scr[0:1, 3 * D:4 * D]

        def x1_of(r):
            rows = pl.ds(pl.multiple_of(r * BF, BF), BF)
            return x_v[rows, :].astype(F32) + ga * acc_scr[rows, :]

        def pre(r, h2_ref):
            h2_ref[...] = (_ln(x1_of(r)) * cb1 + sb).astype(BF16)

        def ffn(r, h2_ref):
            rows = pl.ds(pl.multiple_of(r * BF, BF), BF)
            h2 = h2_ref[...]
            g = jnp.dot(h2, wg_v[...], preferred_element_type=F32)
            u = jnp.dot(h2, wu_v[...], preferred_element_type=F32)
            a = (_gelu(g) * u).astype(BF16)
            y = jnp.dot(a, wd_v[...], preferred_element_type=F32)
            o_v[rows, :] = (x1_of(r) + gb * y).astype(BF16)

        pre(0, h2a_scr)

        def fbody(rr, carry):
            r = 2 * rr
            ffn(r, h2a_scr)
            cp_o(r).start()
            pre(r + 1, h2b_scr)
            ffn(r + 1, h2b_scr)
            pre(jnp.minimum(r + 2, NF - 1), h2a_scr)
            cp_o(r + 1).start()
            return carry

        jax.lax.fori_loop(0, NF // 2, fbody, 0)

        def wbody(r, carry):
            cp_o(r).wait()
            return carry

        jax.lax.fori_loop(0, NF, wbody, 0)

    x2 = A_x.reshape(S, D)
    k3 = A_k_cache.reshape(H, SK, DH)
    v3 = A_v_cache.reshape(H, SK, DH)
    hbm = pl.BlockSpec(memory_space=pl.ANY)
    out = pl.pallas_call(
        kernel,
        in_specs=[hbm] * 10,
        out_specs=hbm,
        out_shape=jax.ShapeDtypeStruct((S, D), BF16),
        scratch_shapes=[
            pltpu.VMEM((S, D), BF16),
            pltpu.VMEM((1, D), BF16),
            pltpu.VMEM((D, 6 * D), BF16),
            pltpu.VMEM((2, D, DH), BF16),
            pltpu.VMEM((2, SK, DH), BF16),
            pltpu.VMEM((2, SK, DH), BF16),
            pltpu.VMEM((2, DH, D), BF16),
            pltpu.VMEM((D, FF), BF16),
            pltpu.VMEM((D, FF), BF16),
            pltpu.VMEM((FF, D), BF16),
            pltpu.VMEM((S, D), BF16),
            pltpu.VMEM((S, D), F32),
            pltpu.VMEM((S, DH), BF16),
            pltpu.VMEM((8, 4 * D), F32),
            pltpu.VMEM((S, D), BF16),
            pltpu.VMEM((BF, D), BF16),
            pltpu.VMEM((BF, D), BF16),
            pltpu.VMEM((R, DH), F32),
            pltpu.VMEM((R, DH), F32),
            pltpu.SemaphoreType.DMA((XCH,)),
            pltpu.SemaphoreType.DMA((3,)),
            pltpu.SemaphoreType.DMA((4, 2)),
            pltpu.SemaphoreType.DMA((3,)),
            pltpu.SemaphoreType.DMA((NF,)),
        ],
        compiler_params=pltpu.CompilerParams(vmem_limit_bytes=100 * 1024 * 1024),
    )(x2, c, w_mod, A_wq, k3, v3, A_wo, B_w_gate, B_w_up, B_w_down)
    return out.reshape(B, S, D)
```
